```python
import jax
import jax.numpy as jnp

def _softmax(x, axis=-1):
    return jax.nn.softmax(x, axis=axis)

def _gelu(x):
    return jax.nn.gelu(x, approximate=True)

def _silu(x):
    return jax.nn.silu(x)

def _sigmoid(x):
    return jax.nn.sigmoid(x)

def _layernorm(x, axis=-1, eps=1e-05):
    m = jnp.mean(x, axis=axis, keepdims=True)
    v = jnp.var(x, axis=axis, keepdims=True)
    return (x - m) / jnp.sqrt(v + eps)

def _scatter_add(tgt, idx, src, axis=0):
    return tgt.at[idx].add(src)

def _segment_sum(src, seg, n):
    return jax.ops.segment_sum(src, seg, n)

class _Rng:

    def __init__(self, key):
        self._k = key

    def _next(self):
        self._k, sub = jax.random.split(self._k)
        return sub

    def normal(self, shape):
        return jax.random.normal(self._next(), shape, dtype=jnp.bfloat16)

    def randint(self, lo, hi, shape):
        return jax.random.randint(self._next(), shape, lo, hi, dtype=jnp.int32)

    def uniform(self, shape, lo=0.0, hi=1.0):
        return jax.random.uniform(self._next(), shape, jnp.bfloat16, lo, hi)

    def permutation(self, n):
        return jax.random.permutation(self._next(), n)
kernel_name = 'interleave_layers__memory_aug_infini_attn__mixer_s_mlp__prompt'

def setup_inputs():
    _rng = _Rng(jax.random.key(int.from_bytes(__import__("os").urandom(4), "little")))
    _w = lambda a: (lambda t: t.astype(jnp.bfloat16) if jnp.issubdtype(t.dtype, jnp.floating) else t)(jnp.asarray(a))

    def _A_setup():
        B, S, D, H = (1, 2048, 1024, 32)
        N = 4
        L = max(1, S // N)
        sc = D ** (-0.5)
        return {'x': _w((lambda *s: _rng.normal(s) * 0.05)(B, N * L, D)), 'wq': _w((lambda *s: _rng.normal(s) * 0.05)(D, D) * sc), 'wk': _w((lambda *s: _rng.normal(s) * 0.05)(D, D) * sc), 'wv': _w((lambda *s: _rng.normal(s) * 0.05)(D, D) * sc), 'wo': _w((lambda *s: _rng.normal(s) * 0.05)(D, D) * sc), 'beta': _w((lambda *s: _rng.normal(s) * 0.05)(H))}
    _A_in = _A_setup()

    def _B_setup():
        B, S, D, F = (1, 2048, 1024, 3584)
        return {'x': _w((lambda *s: _rng.normal(s) * 0.05)(B, S, D)), 'w1': _w((lambda *s: _rng.normal(s) * 0.05)(D, D) * D ** (-0.5)), 'w2': _w((lambda *s: _rng.normal(s) * 0.05)(D, D) * D ** (-0.5)), 'w3': _w((lambda *s: _rng.normal(s) * 0.05)(D, F) * D ** (-0.5)), 'w4': _w((lambda *s: _rng.normal(s) * 0.05)(F, D) * F ** (-0.5))}
    _B_in = _B_setup()
    return {'A_x': _A_in['x'], 'A_wq': _A_in['wq'], 'A_wk': _A_in['wk'], 'A_wv': _A_in['wv'], 'A_wo': _A_in['wo'], 'A_beta': _A_in['beta'], 'B_x': _B_in['x'], 'B_w1': _B_in['w1'], 'B_w2': _B_in['w2'], 'B_w3': _B_in['w3'], 'B_w4': _B_in['w4']}

def reference(A_x, A_wq, A_wk, A_wv, A_wo, A_beta, B_x, B_w1, B_w2, B_w3, B_w4):

    def _A_ref(x, wq, wk, wv, wo, beta):
        B, S, D = x.shape
        H = 32
        Dh = D // H
        N = 4
        L = S // N
        q = (lambda x, *d: x.transpose(*d))((x @ wq).reshape(B, S, H, Dh), 0, 2, 1, 3).reshape(B, H, N, L, Dh)
        k = (lambda x, *d: x.transpose(*d))((x @ wk).reshape(B, S, H, Dh), 0, 2, 1, 3).reshape(B, H, N, L, Dh)
        v = (lambda x, *d: x.transpose(*d))((x @ wv).reshape(B, S, H, Dh), 0, 2, 1, 3).reshape(B, H, N, L, Dh)
        phi = lambda t: jnp.where(t > 0, t + 1.0, jnp.exp(t))
        scale = Dh ** (-0.5)
        ar = jnp.arange(L)
        mask = (lambda x, dt: x.astype(dt))(ar[:, None] < ar[None, :], x.dtype) * -1000000000.0
        g = _sigmoid(beta).reshape(1, H, 1, 1)
        M = jnp.einsum('bhd,bhe->bhde', q[:, :, 0, 0, :] * 0.0, q[:, :, 0, 0, :] * 0.0)
        z = q[:, :, 0, 0, :] * 0.0
        outs = []
        for s in range(N):
            qs, ks, vs = (q[:, :, s].copy(), k[:, :, s].copy(), v[:, :, s].copy())
            logits = jnp.einsum('bhqd,bhkd->bhqk', qs, ks) * scale + mask
            p = _softmax(logits, axis=-1)
            a_dot = jnp.einsum('bhqk,bhkd->bhqd', p, vs)
            pq = phi(qs)
            num = jnp.einsum('bhld,bhde->bhle', pq, M)
            den = jnp.einsum('bhld,bhd->bhl', pq, z)[..., None] + 1e-06
            a_mem = num / den
            o = g * a_mem + (1.0 - g) * a_dot
            outs.append(o)
            pk = phi(ks)
            M = M + jnp.einsum('bhld,bhle->bhde', pk, vs)
            z = z + jnp.einsum('bhld->bhd', pk)
        o = (lambda x, *d: x.transpose(*d))(jnp.stack(outs, 2).reshape(B, H, S, Dh), 0, 2, 1, 3).reshape(B, S, D)
        return o @ wo

    def _B_ref(x, w1, w2, w3, w4):
        B, S, D = x.shape
        h = _gelu(_layernorm(x, axis=-1) @ w1)
        c = D // 4
        g0 = jnp.pad(h[:, :, 0 * c:1 * c], ((0, 0), (1, 0), (0, 0)))[:, :S, :]
        g1 = jnp.pad(h[:, :, 1 * c:2 * c], ((0, 0), (0, 1), (0, 0)))[:, 1:, :]
        g2 = jnp.pad(h[:, :, 2 * c:3 * c], ((0, 0), (2, 0), (0, 0)))[:, :S, :]
        g3 = jnp.pad(h[:, :, 3 * c:], ((0, 0), (0, 2), (0, 0)))[:, 2:, :]
        hs = jnp.concatenate([g0, g1, g2, g3], axis=-1) @ w2
        x1 = x + hs
        h2 = _gelu(_layernorm(x1, axis=-1) @ w3) @ w4
        return x1 + h2
    x = A_x
    x = x + _A_ref(_layernorm(x, axis=-1), A_wq, A_wk, A_wv, A_wo, A_beta)
    x = x + _B_ref(_layernorm(x, axis=-1), B_w1, B_w2, B_w3, B_w4)
    x = x + _A_ref(_layernorm(x, axis=-1), A_wq, A_wk, A_wv, A_wo, A_beta)
    x = x + _B_ref(_layernorm(x, axis=-1), B_w1, B_w2, B_w3, B_w4)
    return x
```

```python
import math
import jax
import jax.numpy as jnp
from jax import lax
import jax.experimental.pallas as pl
import jax.experimental.pallas.tpu as pltpu

S, D, H, DH, NSEG, L, F = 2048, 1024, 32, 32, 4, 512, 3584
NG = D // 128
EPS = 1e-5
NT = (((1,), (1,)), ((), ()))
QSCALE = (DH ** -0.5) * math.log2(math.e)
DEPTH = 8


def _ln(x):
    m = jnp.mean(x, axis=-1, keepdims=True)
    d = x - m
    v = jnp.mean(d * d, axis=-1, keepdims=True)
    return d * lax.rsqrt(v + EPS)


def _gelu(x):
    c = math.sqrt(2.0 / math.pi)
    return 0.5 * x * (1.0 + jnp.tanh(c * (x + 0.044715 * (x * x * x))))


def _phi(t):
    return jnp.where(t > 0, t + 1.0, jnp.exp(t))


def _dot(a, b):
    return jnp.dot(a, b, preferred_element_type=jnp.float32)


def _dot_nt(a, b):
    return lax.dot_general(a, b, NT, preferred_element_type=jnp.float32)


def _kernel(x_hbm, wq_hbm, wk_hbm, wv_hbm, wo_hbm, beta_ref, w1_hbm, w2_hbm, w3_hbm, w4_hbm,
            out_hbm,
            wq, wk, wv, wo, w1, w2, w3, w4,
            xio, xres, xn_s, hbuf, q_s, pq_s, k_s, pk_s, vT_s, o_s, mT_s, z_s, nd_s, g_s, u_s,
            sem_w, sem_x, sem_o):
    bf16, f32 = jnp.bfloat16, jnp.float32

    x_cp = [pltpu.make_async_copy(x_hbm.at[pl.ds(s * L, L)], xio.at[pl.ds(s * L, L)], sem_x.at[s])
            for s in range(NSEG)]
    w_cp = [pltpu.make_async_copy(a, b, sem_w.at[i]) for i, (a, b) in enumerate(
        [(wq_hbm, wq), (wk_hbm, wk), (wv_hbm, wv), (wo_hbm, wo), (w1_hbm, w1), (w2_hbm, w2),
         (w3_hbm, w3), (w4_hbm, w4)])]
    x_cp[0].start()
    for i in range(3):
        w_cp[i].start()
    for s in range(1, NSEG):
        x_cp[s].start()
    for i in range(3, 8):
        w_cp[i].start()

    lane = lax.broadcasted_iota(jnp.int32, (128, 128), 1)
    row = lax.broadcasted_iota(jnp.int32, (128, 128), 0)
    maskT = jnp.where(row > lane, -1e9, 0.0).astype(f32)
    maskT4 = jnp.concatenate([maskT] * 4, axis=1)
    bd = (row // DH) == (lane // DH)
    lane64 = lax.broadcasted_iota(jnp.int32, (64, 128), 1)
    zrow = lax.broadcasted_iota(jnp.int32, (32, 128), 0)
    zlane = lax.broadcasted_iota(jnp.int32, (32, 128), 1)
    zmask = (zrow // 8) == (zlane // DH)

    gv = jax.nn.sigmoid(beta_ref[...].astype(f32))
    hl = lax.broadcasted_iota(jnp.int32, (1, H), 1)
    for h in range(H):
        gh = jnp.sum(jnp.where(hl == h, gv, 0.0), axis=1, keepdims=True)
        g_s[h] = jnp.broadcast_to(gh, (8, 128))

    hbuf[0:8, :] = jnp.zeros((8, D), f32)
    hbuf[8 + S:16 + S, :] = jnp.zeros((8, D), f32)

    def qk(st, g, i, j):
        c = slice(128 * g, 128 * (g + 1))
        q4u = pltpu.bitcast(q_s[128 * i:128 * (i + 1), c], jnp.uint32)
        qm = jnp.concatenate(
            [pltpu.bitcast(jnp.where(lane64 // DH == h, q4u, jnp.uint32(0)), bf16) for h in range(4)],
            axis=0)
        s = _dot_nt(k_s[128 * j:128 * (j + 1), c], qm)
        if j == i:
            s = s + maskT4
        mx = jnp.max(s.reshape(16, 8, 512), axis=0)
        e = st.setdefault((g, i), {'blocks': {}, 'm': None, 'acc': [None] * 4, 'l': [None] * 4})
        e['blocks'][j] = s
        e['m'] = mx if e['m'] is None else jnp.maximum(e['m'], mx)
        if j == i:
            e['m'] = jnp.max(e['m'], axis=0, keepdims=True)

    def pv(st, g, i, j):
        e = st[(g, i)]
        m = e['m']
        acc = e['acc']
        for h in range(4):
            pf = jnp.exp2(e['blocks'][j][:, 128 * h:128 * (h + 1)] - m[:, 128 * h:128 * (h + 1)])
            ls = jnp.sum(pf.reshape(16, 8, 128), axis=0)
            e['l'][h] = ls if e['l'][h] is None else e['l'][h] + ls
            t = _dot(vT_s[128 * g + 32 * h:128 * g + 32 * h + 32, 128 * j:128 * (j + 1)], pf.astype(bf16))
            acc[h] = t if acc[h] is None else acc[h] + t
        if j == i:
            outs = []
            for h in range(4):
                l = jnp.sum(e['l'][h], axis=0, keepdims=True)
                a_dot = acc[h] * pltpu.reciprocal(l, approx=True)
                num = nd_s[g, 32 * h:32 * h + 32, 128 * i:128 * (i + 1)]
                den = nd_s[g, 128 + 8 * h:128 + 8 * h + 8, 128 * i:128 * (i + 1)] + 1e-6
                rden = jnp.concatenate([pltpu.reciprocal(den, approx=True)] * 4, axis=0)
                gg = jnp.concatenate([g_s[4 * g + h]] * 4, axis=0)
                outs.append(gg * (num * rden) + (1.0 - gg) * a_dot)
            oT = jnp.concatenate(outs, axis=0)
            o_s[128 * i:128 * (i + 1), 128 * g:128 * (g + 1)] = oT.T.astype(bf16)
            del st[(g, i)]

    def a_block(rep, s):
        r0 = pl.multiple_of(s * L, L)

        @pl.when(rep == 0)
        def _():
            for ss in range(NSEG):
                @pl.when(s == ss)
                def _():
                    x_cp[ss].wait()
            xres[pl.ds(r0, L), :] = xio[pl.ds(r0, L), :].astype(f32)

        @pl.when(jnp.logical_and(rep == 0, s == 0))
        def _():
            for i in range(3):
                w_cp[i].wait()

        @pl.when(s == 0)
        def _():
            mT_s[...] = jnp.zeros_like(mT_s)
            z_s[...] = jnp.zeros_like(z_s)

        x = xres[pl.ds(r0, L), :]
        xn = _ln(x).astype(bf16)
        q = _dot(xn, wq[...])
        q_s[...] = (q * QSCALE).astype(bf16)
        pq_s[...] = _phi(q).astype(bf16)
        k = _dot(xn, wk[...])
        k_s[...] = k.astype(bf16)
        pk = _phi(k)
        pk_s[...] = pk.astype(bf16)
        zadd = jnp.sum(pk.reshape(L // 8, 8, D), axis=0)
        v = _dot(xn, wv[...]).astype(bf16)
        vT_s[...] = v.T

        for g in range(NG):
            c = slice(128 * g, 128 * (g + 1))
            mT = jnp.where(bd, mT_s[g], 0.0).astype(bf16)
            zr = jnp.where(zmask, jnp.broadcast_to(z_s[0:1, c], (32, 128)), 0.0).astype(bf16)
            lhs = jnp.concatenate([mT, zr], axis=0)
            nd_s[g] = _dot_nt(lhs, pq_s[:, c])
        for g in range(NG):
            c = slice(128 * g, 128 * (g + 1))
            mT_s[g] = mT_s[g] + _dot(vT_s[c, :], pk_s[:, c])
        z_s[0:1, :] = z_s[0:1, :] + jnp.sum(zadd, axis=0, keepdims=True)

        items = [(g, i, j) for g in range(NG) for i in range(4) for j in range(i + 1)]
        st = {}
        for t in range(len(items) + DEPTH):
            if t < len(items):
                qk(st, *items[t])
            if t - DEPTH >= 0:
                pv(st, *items[t - DEPTH])

        @pl.when(jnp.logical_and(rep == 0, s == 0))
        def _():
            w_cp[3].wait()
            w_cp[4].wait()

        x = xres[pl.ds(r0, L), :] + _dot(o_s[...], wo[...])
        xres[pl.ds(r0, L), :] = x
        xn = _ln(x)
        xn_s[pl.ds(r0, L), :] = xn
        hh = _gelu(_dot(_ln(xn).astype(bf16), w1[...]))
        hbuf[pl.ds(pl.multiple_of(r0 + 8, 8), L), :] = hh

    def b_block(rep, b):
        r0 = pl.multiple_of(b * L, L)

        @pl.when(jnp.logical_and(rep == 0, b == 0))
        def _():
            for i in range(5, 8):
                w_cp[i].wait()

        parts = []
        for gi, off in enumerate((7, 9, 6, 10)):
            win = hbuf[pl.ds(r0, L + 16), 256 * gi:256 * (gi + 1)]
            parts.append(win[off:off + L].astype(bf16))
        hs = _dot(jnp.concatenate(parts, axis=1), w2[...])
        x1 = xn_s[pl.ds(r0, L), :] + hs
        u_s[...] = _gelu(_dot(_ln(x1).astype(bf16), w3[...])).astype(bf16)
        y = xres[pl.ds(r0, L), :] + (x1 + _dot(u_s[...], w4[...]))
        xres[pl.ds(r0, L), :] = y

        @pl.when(rep == 1)
        def _():
            xio[pl.ds(r0, L), :] = y.astype(bf16)
            for bb in range(NSEG):
                @pl.when(b == bb)
                def _():
                    pltpu.make_async_copy(xio.at[pl.ds(bb * L, L)], out_hbm.at[pl.ds(bb * L, L)],
                                          sem_o.at[bb]).start()

    def rep_body(rep, carry):
        lax.fori_loop(0, NSEG, lambda s, c: (a_block(rep, s), c)[1], 0)
        lax.fori_loop(0, NSEG, lambda b, c: (b_block(rep, b), c)[1], 0)
        return carry

    lax.fori_loop(0, 2, rep_body, 0)
    for bb in range(NSEG):
        pltpu.make_async_copy(xio.at[pl.ds(bb * L, L)], out_hbm.at[pl.ds(bb * L, L)],
                              sem_o.at[bb]).wait()


@jax.jit
def pallas_interleave_layers__memory_aug_infini_attn__mixer_s_mlp__prompt_kernel(
        A_x, A_wq, A_wk, A_wv, A_wo, A_beta, B_x, B_w1, B_w2, B_w3, B_w4):
    bf16, f32 = jnp.bfloat16, jnp.float32
    V = pltpu.VMEM
    hbm = pl.BlockSpec(memory_space=pl.ANY)
    scratch = [
        V((D, D), bf16), V((D, D), bf16), V((D, D), bf16), V((D, D), bf16),
        V((D, D), bf16), V((D, D), bf16), V((D, F), bf16), V((F, D), bf16),
        V((S, D), bf16),
        V((S, D), f32),
        V((S, D), f32),
        V((S + 16, D), f32),
        V((L, D), bf16), V((L, D), bf16), V((L, D), bf16), V((L, D), bf16),
        V((D, L), bf16),
        V((L, D), bf16),
        V((NG, 128, 128), f32),
        V((8, D), f32),
        V((NG, 160, L), f32),
        V((H, 8, 128), f32),
        V((L, F), bf16),
        pltpu.SemaphoreType.DMA((8,)), pltpu.SemaphoreType.DMA((NSEG,)),
        pltpu.SemaphoreType.DMA((NSEG,)),
    ]
    out = pl.pallas_call(
        _kernel,
        out_shape=jax.ShapeDtypeStruct((S, D), bf16),
        in_specs=[hbm, hbm, hbm, hbm, hbm, pl.BlockSpec(memory_space=pltpu.VMEM), hbm, hbm, hbm, hbm],
        out_specs=hbm,
        scratch_shapes=scratch,
        compiler_params=pltpu.CompilerParams(vmem_limit_bytes=120 * 2 ** 20),
        name="fused",
    )(A_x.reshape(S, D), A_wq, A_wk, A_wv, A_wo, A_beta.reshape(1, H), B_w1, B_w2, B_w3, B_w4)
    return out.reshape(1, S, D)
```

```python
import math
import jax
import jax.numpy as jnp
from jax import lax
import jax.experimental.pallas as pl
import jax.experimental.pallas.tpu as pltpu

S, D, H, DH, NSEG, L, F = 2048, 1024, 32, 32, 4, 512, 3584
NG = D // 128
EPS = 1e-5
NT = (((1,), (1,)), ((), ()))
QSCALE = (DH ** -0.5) * math.log2(math.e)
DEPTH = 8
RB = 512
NB = 256
NB4 = 128
NREP = 2
LAG = 2


def _ln(x):
    m = jnp.mean(x, axis=-1, keepdims=True)
    d = x - m
    v = jnp.mean(d * d, axis=-1, keepdims=True)
    return d * lax.rsqrt(v + EPS)


def _gelu(x):
    c = math.sqrt(2.0 / math.pi)
    return 0.5 * x * (1.0 + jnp.tanh(c * (x + 0.044715 * (x * x * x))))


def _phi(t):
    return jnp.where(t > 0, t + 1.0, jnp.exp(t))


def _dot(a, b):
    return jnp.dot(a, b, preferred_element_type=jnp.float32)


def _dot_nt(a, b):
    return lax.dot_general(a, b, NT, preferred_element_type=jnp.float32)


def _merge(streams):
    streams = [(gen, total) for gen, total in streams]
    done = [0.0] * len(streams)
    alive = [True] * len(streams)
    while any(alive):
        best = None
        for i, (gen, total) in enumerate(streams):
            if alive[i] and (best is None or done[i] / total < done[best] / streams[best][1]):
                best = i
        try:
            done[best] += next(streams[best][0])
        except StopIteration:
            alive[best] = False


def _kernel(x_hbm, wq_hbm, wk_hbm, wv_hbm, wo_hbm, beta_ref, w1_hbm, w2_hbm, w3_hbm, w4_hbm,
            out_hbm,
            wq, wk, wv, wo, w1, w2, w3, w4,
            xio, xres, xn_s, hbuf, xa_s, q_s, pq_s, k_s, pk_s, vT_s, o_s, xb_s, mT_s, z_s, nd_s, g_s,
            hs_s, x1_s, x1n_s, u_s,
            sem_w, sem_x, sem_o):
    bf16, f32 = jnp.bfloat16, jnp.float32

    x_cp = [pltpu.make_async_copy(x_hbm.at[pl.ds(s * L, L)], xio.at[pl.ds(s * L, L)], sem_x.at[s])
            for s in range(NSEG)]
    w_cp = [pltpu.make_async_copy(a, b, sem_w.at[i]) for i, (a, b) in enumerate(
        [(wq_hbm, wq), (wk_hbm, wk), (wv_hbm, wv), (wo_hbm, wo), (w1_hbm, w1), (w2_hbm, w2),
         (w3_hbm, w3), (w4_hbm, w4)])]
    x_cp[0].start()
    for i in range(3):
        w_cp[i].start()
    for s in range(1, NSEG):
        x_cp[s].start()
    for i in range(3, 8):
        w_cp[i].start()

    lane = lax.broadcasted_iota(jnp.int32, (128, 128), 1)
    row = lax.broadcasted_iota(jnp.int32, (128, 128), 0)
    maskT = jnp.where(row > lane, -1e9, 0.0).astype(f32)
    maskT4 = jnp.concatenate([maskT] * 4, axis=1)
    bd = (row // DH) == (lane // DH)
    lane64 = lax.broadcasted_iota(jnp.int32, (64, 128), 1)
    zrow = lax.broadcasted_iota(jnp.int32, (32, 128), 0)
    zlane = lax.broadcasted_iota(jnp.int32, (32, 128), 1)
    zmask = (zrow // 8) == (zlane // DH)

    gv = jax.nn.sigmoid(beta_ref[...].astype(f32))
    hl = lax.broadcasted_iota(jnp.int32, (1, H), 1)
    for h in range(H):
        gh = jnp.sum(jnp.where(hl == h, gv, 0.0), axis=1, keepdims=True)
        g_s[h] = jnp.broadcast_to(gh, (8, 128))

    hbuf[0:8, :] = jnp.zeros((8, D), f32)
    hbuf[8 + S:16 + S, :] = jnp.zeros((8, D), f32)

    def rows(r0, off, n):
        if isinstance(r0, int):
            return pl.ds(r0 + off, n)
        return pl.ds(pl.multiple_of(r0 + off, 8), n)

    def qmask(q4):
        q4u = pltpu.bitcast(q4, jnp.uint32)
        return [pltpu.bitcast(jnp.where(lane64 // DH == h, q4u, jnp.uint32(0)), bf16) for h in range(4)]

    def combine(g, i, h, a_dot, use_mem, c, qr):
        gg = jnp.concatenate([g_s[4 * g + h]] * 4, axis=0)
        if use_mem:
            num = nd_s[g, 32 * h:32 * h + 32, qr]
            den = nd_s[g, 128 + 8 * h:128 + 8 * h + 8, qr] + 1e-6
            rden = jnp.concatenate([pltpu.reciprocal(den, approx=True)] * 4, axis=0)
            return gg * (num * rden) + (1.0 - gg) * a_dot
        return (1.0 - gg) * a_dot

    def qk(st, g, i, j):
        c = slice(128 * g, 128 * (g + 1))
        qm = jnp.concatenate(qmask(q_s[128 * i:128 * (i + 1), c]), axis=0)
        s = _dot_nt(k_s[128 * j:128 * (j + 1), c], qm)
        if j == i:
            s = s + maskT4
        e = st.setdefault((g, i), {'blocks': {}, 'acc': [None] * 4, 'l': [None] * 4})
        e['blocks'][j] = s

    def pv(st, g, i, j, use_mem):
        e = st[(g, i)]
        acc = e['acc']
        for h in range(4):
            pf = jnp.exp2(e['blocks'][j][:, 128 * h:128 * (h + 1)])
            ls = jnp.sum(pf.reshape(16, 8, 128), axis=0)
            e['l'][h] = ls if e['l'][h] is None else e['l'][h] + ls
            t = _dot(vT_s[128 * g + 32 * h:128 * g + 32 * h + 32, 128 * j:128 * (j + 1)], pf.astype(bf16))
            acc[h] = t if acc[h] is None else acc[h] + t
        if j == i:
            outs = []
            for h in range(4):
                l = jnp.sum(e['l'][h], axis=0, keepdims=True)
                a_dot = acc[h] * pltpu.reciprocal(l, approx=True)
                outs.append(combine(g, i, h, a_dot, use_mem, None, slice(128 * i, 128 * (i + 1))))
            oT = jnp.concatenate(outs, axis=0)
            o_s[128 * i:128 * (i + 1), 128 * g:128 * (g + 1)] = oT.T.astype(bf16)
            del st[(g, i)]

    def attn_safe_path(use_mem):
        def grp(g, carry):
            c = pl.ds(pl.multiple_of(g * 128, 128), 128)
            for i in range(4):
                nk = 128 * (i + 1)
                qr = slice(128 * i, 128 * (i + 1))
                qms = qmask(q_s[qr, c])
                outs = []
                for h in range(4):
                    sT = _dot_nt(k_s[0:nk, c], qms[h])
                    if i > 0:
                        sT = jnp.concatenate([sT[:nk - 128], sT[nk - 128:] + maskT], axis=0)
                    else:
                        sT = sT + maskT
                    m = jnp.max(sT, axis=0, keepdims=True)
                    pf = jnp.exp2(sT - m)
                    l = jnp.sum(pf, axis=0, keepdims=True)
                    vr = pl.ds(pl.multiple_of(g * 128 + 32 * h, 32), 32)
                    a_dot = _dot(vT_s[vr, 0:nk], pf.astype(bf16)) / l
                    outs.append(combine(g, i, h, a_dot, use_mem, c, qr))
                o_s[qr, c] = jnp.concatenate(outs, axis=0).T.astype(bf16)
            return carry
        lax.fori_loop(0, NG, grp, 0)

    def conv_x(s):
        x_cp[s].wait()
        for r in range(0, L, 256):
            rr = slice(s * L + r, s * L + r + 256)
            x = xio[rr, :].astype(f32)
            xres[rr, :] = x
            xa_s[rr, :] = _ln(x).astype(bf16)

    def out_cp(b):
        return pltpu.make_async_copy(xio.at[pl.ds(b * L, L)], out_hbm.at[pl.ds(b * L, L)], sem_o.at[b])

    def hs_prep(b):
        r0 = b * L
        for gi, off in enumerate((7, 9, 6, 10)):
            c = slice(256 * gi, 256 * (gi + 1))
            win = hbuf[r0:r0 + L + 16, c]
            hs_s[r0:r0 + L, c] = win[off:off + L].astype(bf16)

    def ln2(r0, r, n):
        xn = _ln(xres[r0 + r:r0 + r + n, :])
        xn_s[r0 + r:r0 + r + n, :] = xn
        xb_s[r:r + n, :] = _ln(xn).astype(bf16)

    def vmaxacc(acc, t):
        n, w = t.shape
        m = jnp.max(jnp.abs(t).reshape(n // 8, 8, w), axis=0)
        m = jnp.maximum(m[:, :128], m[:, 128:]) if w == 256 else m
        return m if acc is None else jnp.maximum(acc, m)

    def a_block(rep, s, hooks):
        r0 = s * L
        use_mem = s > 0
        do_upd = s < NSEG - 1

        def hook(name):
            for f in hooks.pop(name, []):
                f()
        zparts = []
        qmx = kmx = None
        for ci, c0 in enumerate(range(0, D, NB)):
            c = slice(c0, c0 + NB)
            lhs = xa_s[r0:r0 + L, :]
            q = _dot(lhs, wq[:, c])
            qs = q * QSCALE
            q_s[:, c] = qs.astype(bf16)
            qmx = vmaxacc(qmx, qs)
            if use_mem:
                pq_s[:, c] = _phi(q).astype(bf16)
            hook(('q', ci))
            k = _dot(lhs, wk[:, c])
            k_s[:, c] = k.astype(bf16)
            kmx = vmaxacc(kmx, k)
            if do_upd:
                pk = _phi(k)
                pk_s[:, c] = pk.astype(bf16)
                zparts.append(jnp.sum(pk.reshape(L // 8, 8, NB), axis=0))
            hook(('k', ci))
            v = _dot(lhs, wv[:, c]).astype(bf16)
            vT_s[c, :] = v.T
            hook(('v', ci))
        bound = jnp.max(qmx) * jnp.max(kmx) * (DH * 1.02)
        safe = bound <= 60.0
        if do_upd:
            znew = jnp.sum(jnp.concatenate(zparts, axis=1), axis=0, keepdims=True)
        for g in range(NG):
            c = slice(128 * g, 128 * (g + 1))
            if use_mem:
                m_old = mT_s[g]
                z_old = z_s[0:1, c]
                mT = jnp.where(bd, m_old, 0.0).astype(bf16)
                zr = jnp.where(zmask, jnp.broadcast_to(z_old, (32, 128)), 0.0).astype(bf16)
                lhs = jnp.concatenate([mT, zr], axis=0)
                nd_s[g] = _dot_nt(lhs, pq_s[:, c])
            if do_upd:
                upd = _dot(vT_s[c, :], pk_s[:, c])
                if use_mem:
                    mT_s[g] = m_old + upd
                    z_s[0:1, c] = z_old + znew[:, c]
                else:
                    mT_s[g] = upd
                    z_s[0:1, c] = znew[:, c]
        items = [(g, i, j) for g in range(NG) for i in range(4) for j in range(i + 1)]
        st = {}
        for t in range(len(items) + DEPTH):
            if t < len(items):
                qk(st, *items[t])
            if t - DEPTH >= 0:
                pv(st, *items[t - DEPTH], use_mem)
            hook(('att', t))
        hook('att_end')

        @pl.when(jnp.logical_not(safe))
        def _():
            attn_safe_path(use_mem)
        HF = L // 2
        for r in (0, HF):
            for c0 in range(0, D, NB):
                c = slice(c0, c0 + NB)
                xres[r0 + r:r0 + r + HF, c] = xres[r0 + r:r0 + r + HF, c] + _dot(o_s[r:r + HF, :], wo[:, c])
        ln2(r0, 0, HF)
        for r in (0, HF):
            for c0 in range(0, D, NB):
                c = slice(c0, c0 + NB)
                hbuf[8 + r0 + r:8 + r0 + r + HF, c] = _gelu(_dot(xb_s[r:r + HF, :], w1[:, c]))
                if r == 0 and c0 == 0:
                    ln2(r0, HF, HF)
            hook(('w1', r))
        assert not hooks, hooks

    def b_block(final, b, hooks):
        r0 = b * L
        HF = L // 2

        def hook(name):
            for f in hooks.pop(name, []):
                f()
        for r in (0, HF):
            for c0 in range(0, D, NB):
                c = slice(c0, c0 + NB)
                x1_s[r:r + HF, c] = xn_s[r0 + r:r0 + r + HF, c] + _dot(hs_s[r0 + r:r0 + r + HF, :], w2[:, c])
                hook(('w2', r, c0))
        x1n_s[0:HF, :] = _ln(x1_s[0:HF, :]).astype(bf16)
        for c0 in range(0, F, NB):
            c = slice(c0, c0 + NB)
            if c0 == 0:
                u_s[0:HF, c] = _gelu(_dot(x1n_s[0:HF, :], w3[:, c])).astype(bf16)
                x1n_s[HF:L, :] = _ln(x1_s[HF:L, :]).astype(bf16)
                u_s[HF:L, c] = _gelu(_dot(x1n_s[HF:L, :], w3[:, c])).astype(bf16)
            else:
                u_s[:, c] = _gelu(_dot(x1n_s[...], w3[:, c])).astype(bf16)
        for c0 in range(0, D, NB4):
            c = slice(c0, c0 + NB4)
            y = xres[r0:r0 + L, c] + (x1_s[:, c] + _dot(u_s[...], w4[:, c]))
            if not final:
                xres[r0:r0 + L, c] = y
            else:
                xio[r0:r0 + L, c] = y.astype(bf16)
            hook(('w4', c0))
        assert not hooks, hooks

    def ln_a(b):
        for r in range(0, L, 256):
            rr = slice(b * L + r, b * L + r + 256)
            xa_s[rr, :] = _ln(xres[rr, :]).astype(bf16)

    def wait_w(*idx):
        for i in idx:
            w_cp[i].wait()

    conv_x(0)
    wait_w(0)
    for rep in range(NREP):
        for s in range(NSEG):
            hk = {}
            if rep == 0 and s == 0:
                hk[('q', 0)] = [lambda: wait_w(1)]
                hk[('k', 0)] = [lambda: wait_w(2)]
                hk[('v', 0)] = [lambda: conv_x(1)]
                hk[('v', 1)] = [lambda: conv_x(2)]
                hk[('v', 2)] = [lambda: conv_x(3)]
                hk['att_end'] = [lambda: wait_w(3, 4)]
            if rep > 0 and s == 0:
                hk[('q', 0)] = [lambda: ln_a(3)]
            if s == NSEG - 1:
                hk[('q', 1)] = [lambda: hs_prep(0)]
                hk[('q', 2)] = [lambda: hs_prep(1)]
            args = (rep, s, hk)
            a_block(*args)
        for b in range(NSEG):
            hk = {}
            if rep == 0 and b == 0:
                wait_w(5, 6, 7)
            if b == 0:
                hk[('w2', 0, 0)] = [lambda: hs_prep(2)]
                hk[('w2', 0, NB)] = [lambda: hs_prep(3)]
            else:
                if rep < NREP - 1:
                    hk[('w2', 0, 0)] = [(lambda bb: lambda: ln_a(bb))(b - 1)]
                else:
                    hk[('w2', 0, 0)] = [(lambda bb: lambda: out_cp(bb).start())(b - 1)]
            b_block(rep == NREP - 1, b, hk)
    if NREP == 2 or True:
        out_cp(NSEG - 1).start()
        for b in range(NSEG):
            out_cp(b).wait()


@jax.jit
def pallas_interleave_layers__memory_aug_infini_attn__mixer_s_mlp__prompt_kernel(
        A_x, A_wq, A_wk, A_wv, A_wo, A_beta, B_x, B_w1, B_w2, B_w3, B_w4):
    bf16, f32 = jnp.bfloat16, jnp.float32
    V = pltpu.VMEM
    hbm = pl.BlockSpec(memory_space=pl.ANY)
    scratch = [
        V((D, D), bf16), V((D, D), bf16), V((D, D), bf16), V((D, D), bf16),
        V((D, D), bf16), V((D, D), bf16), V((D, F), bf16), V((F, D), bf16),
        V((S, D), bf16),
        V((S, D), f32),
        V((S, D), f32),
        V((S + 16, D), f32),
        V((S, D), bf16),
        V((L, D), bf16), V((L, D), bf16), V((L, D), bf16), V((L, D), bf16),
        V((D, L), bf16),
        V((L, D), bf16),
        V((L, D), bf16),
        V((NG, 128, 128), f32),
        V((8, D), f32),
        V((NG, 160, L), f32),
        V((H, 8, 128), f32),
        V((S, D), bf16),
        V((L, D), f32),
        V((L, D), bf16),
        V((L, F), bf16),
        pltpu.SemaphoreType.DMA((8,)), pltpu.SemaphoreType.DMA((NSEG,)),
        pltpu.SemaphoreType.DMA((NSEG,)),
    ]
    out = pl.pallas_call(
        _kernel,
        out_shape=jax.ShapeDtypeStruct((S, D), bf16),
        in_specs=[hbm, hbm, hbm, hbm, hbm, pl.BlockSpec(memory_space=pltpu.VMEM), hbm, hbm, hbm, hbm],
        out_specs=hbm,
        scratch_shapes=scratch,
        compiler_params=pltpu.CompilerParams(vmem_limit_bytes=120 * 2 ** 20),
        name="fused",
    )(A_x.reshape(S, D), A_wq, A_wk, A_wv, A_wo, A_beta.reshape(1, H), B_w1, B_w2, B_w3, B_w4)
    return out.reshape(1, S, D)
```

```python
import math
import jax
import jax.numpy as jnp
from jax import lax
import jax.experimental.pallas as pl
import jax.experimental.pallas.tpu as pltpu

S, D, H, DH, NSEG, L, F = 2048, 1024, 32, 32, 4, 512, 3584
NG = D // 128
EPS = 1e-5
NT = (((1,), (1,)), ((), ()))
QSCALE = (DH ** -0.5) * math.log2(math.e)
DEPTH = 2
RB = 512
NB = 256
NB4 = 128
NREP = 2
LIM = 60.0
IORD = (3, 2, 1, 0)


def _ln(x):
    m = jnp.mean(x, axis=-1, keepdims=True)
    d = x - m
    v = jnp.mean(d * d, axis=-1, keepdims=True)
    return d * lax.rsqrt(v + EPS)


def _gelu(x):
    c = math.sqrt(2.0 / math.pi)
    return 0.5 * x * (1.0 + jnp.tanh(c * (x + 0.044715 * (x * x * x))))


def _phi(t):
    return jnp.where(t > 0, t + 1.0, jnp.exp(t))


def _dot(a, b):
    return jnp.dot(a, b, preferred_element_type=jnp.float32)


def _dot_nt(a, b):
    return lax.dot_general(a, b, NT, preferred_element_type=jnp.float32)


def _merge(streams):
    streams = [(gen, total) for gen, total in streams]
    done = [0.0] * len(streams)
    alive = [True] * len(streams)
    while any(alive):
        best = None
        for i, (gen, total) in enumerate(streams):
            if alive[i] and (best is None or done[i] / total < done[best] / streams[best][1]):
                best = i
        try:
            done[best] += next(streams[best][0])
        except StopIteration:
            alive[best] = False


def _kernel(x_hbm, wq_hbm, wk_hbm, wv_hbm, wo_hbm, beta_ref, w1_hbm, w2_hbm, w3_hbm, w4_hbm,
            out_hbm,
            wq, wk, wv, wo, w1, w2, w3, w4,
            xio, xres, xn_s, hbuf, xa_s, q_s, pq_s, k_s, pk_s, vT_s, o_s, xb_s, mT_s, z_s, nd_s, g_s,
            hs_s, x1_s, x1n_s, u_s,
            sem_w, sem_x, sem_o):
    bf16, f32 = jnp.bfloat16, jnp.float32

    x_cp = [pltpu.make_async_copy(x_hbm.at[pl.ds(s * L, L)], xio.at[pl.ds(s * L, L)], sem_x.at[s])
            for s in range(NSEG)]
    w_cp = [pltpu.make_async_copy(a, b, sem_w.at[i]) for i, (a, b) in enumerate(
        [(wq_hbm, wq), (wk_hbm, wk), (wv_hbm, wv), (wo_hbm, wo), (w1_hbm, w1), (w2_hbm, w2),
         (w3_hbm, w3), (w4_hbm, w4)])]
    x_cp[0].start()
    w_cp[0].start()

    lane = lax.broadcasted_iota(jnp.int32, (128, 128), 1)
    row = lax.broadcasted_iota(jnp.int32, (128, 128), 0)
    maskT = jnp.where(row > lane, -1e9, 0.0).astype(f32)
    maskT4 = jnp.concatenate([maskT] * 4, axis=1)
    bd = (row // DH) == (lane // DH)
    lane64 = lax.broadcasted_iota(jnp.int32, (64, 128), 1)
    zrow = lax.broadcasted_iota(jnp.int32, (32, 128), 0)
    zlane = lax.broadcasted_iota(jnp.int32, (32, 128), 1)
    zmask = (zrow // 8) == (zlane // DH)

    gv = jax.nn.sigmoid(beta_ref[...].astype(f32))
    hl = lax.broadcasted_iota(jnp.int32, (1, H), 1)
    for h in range(H):
        gh = jnp.sum(jnp.where(hl == h, gv, 0.0), axis=1, keepdims=True)
        g_s[h] = jnp.broadcast_to(gh, (8, 128))

    hbuf[0:8, :] = jnp.zeros((8, D), f32)
    hbuf[8 + S:16 + S, :] = jnp.zeros((8, D), f32)

    def rows(r0, off, n):
        if isinstance(r0, int):
            return pl.ds(r0 + off, n)
        return pl.ds(pl.multiple_of(r0 + off, 8), n)

    def qmask(q4):
        q4u = pltpu.bitcast(q4, jnp.uint32)
        return [pltpu.bitcast(jnp.where(lane64 // DH == h, q4u, jnp.uint32(0)), bf16) for h in range(4)]

    def combine(g, i, h, a_dot, use_mem, c, qr):
        gg = jnp.concatenate([g_s[4 * g + h]] * 4, axis=0)
        if use_mem:
            num = nd_s[g, 32 * h:32 * h + 32, qr]
            den = nd_s[g, 128 + 8 * h:128 + 8 * h + 8, qr] + 1e-6
            rden = jnp.concatenate([pltpu.reciprocal(den, approx=True)] * 4, axis=0)
            return gg * (num * rden) + (1.0 - gg) * a_dot
        return (1.0 - gg) * a_dot

    def qk(st, g, i, j):
        c = slice(128 * g, 128 * (g + 1))
        qm = jnp.concatenate(qmask(q_s[128 * i:128 * (i + 1), c]), axis=0)
        s = _dot_nt(k_s[128 * j:128 * (j + 1), c], qm)
        if j == i:
            s = s + maskT4
        e = st.setdefault((g, i), {'blocks': {}, 'acc': [None] * 4, 'l': [None] * 4})
        e['blocks'][j] = s

    def pv(st, g, i, j, use_mem):
        e = st[(g, i)]
        acc = e['acc']
        for h in range(4):
            pf = jnp.exp2(e['blocks'][j][:, 128 * h:128 * (h + 1)])
            ls = jnp.sum(pf.reshape(16, 8, 128), axis=0)
            e['l'][h] = ls if e['l'][h] is None else e['l'][h] + ls
            t = _dot(vT_s[128 * g + 32 * h:128 * g + 32 * h + 32, 128 * j:128 * (j + 1)], pf.astype(bf16))
            acc[h] = t if acc[h] is None else acc[h] + t
        if j == i:
            outs = []
            for h in range(4):
                l = jnp.sum(e['l'][h], axis=0, keepdims=True)
                a_dot = acc[h] * pltpu.reciprocal(l, approx=True)
                outs.append(combine(g, i, h, a_dot, use_mem, None, slice(128 * i, 128 * (i + 1))))
            oT = jnp.concatenate(outs, axis=0)
            o_s[128 * i:128 * (i + 1), 128 * g:128 * (g + 1)] = oT.T.astype(bf16)
            del st[(g, i)]

    def attn_safe_path(use_mem):
        def grp(g, carry):
            c = pl.ds(pl.multiple_of(g * 128, 128), 128)
            for i in range(4):
                nk = 128 * (i + 1)
                qr = slice(128 * i, 128 * (i + 1))
                qms = qmask(q_s[qr, c])
                outs = []
                for h in range(4):
                    sT = _dot_nt(k_s[0:nk, c], qms[h])
                    if i > 0:
                        sT = jnp.concatenate([sT[:nk - 128], sT[nk - 128:] + maskT], axis=0)
                    else:
                        sT = sT + maskT
                    m = jnp.max(sT, axis=0, keepdims=True)
                    pf = jnp.exp2(sT - m)
                    l = jnp.sum(pf, axis=0, keepdims=True)
                    vr = pl.ds(pl.multiple_of(g * 128 + 32 * h, 32), 32)
                    a_dot = _dot(vT_s[vr, 0:nk], pf.astype(bf16)) / l
                    outs.append(combine(g, i, h, a_dot, use_mem, c, qr))
                o_s[qr, c] = jnp.concatenate(outs, axis=0).T.astype(bf16)
            return carry
        lax.fori_loop(0, NG, grp, 0)

    def conv_x(s, wait=True):
        if wait:
            x_cp[s].wait()
        for r in range(0, L, 256):
            rr = slice(s * L + r, s * L + r + 256)
            x = xio[rr, :].astype(f32)
            xres[rr, :] = x
            xa_s[rr, :] = _ln(x).astype(bf16)

    def out_cp(b):
        return pltpu.make_async_copy(xio.at[pl.ds(b * L, L)], out_hbm.at[pl.ds(b * L, L)], sem_o.at[b])

    def hs_prep(b):
        r0 = b * L
        for gi, off in enumerate((7, 9, 6, 10)):
            c = slice(256 * gi, 256 * (gi + 1))
            win = hbuf[r0:r0 + L + 16, c]
            hs_s[r0:r0 + L, c] = win[off:off + L].astype(bf16)

    def ln2(r0, r, n):
        xn = _ln(xres[r0 + r:r0 + r + n, :])
        xn_s[r0 + r:r0 + r + n, :] = xn
        xb_s[r:r + n, :] = _ln(xn).astype(bf16)

    def vmaxacc(acc, t):
        n, w = t.shape
        m = jnp.max(jnp.abs(t).reshape(n // 8, 8, w), axis=0)
        m = jnp.maximum(m[:, :128], m[:, 128:]) if w == 256 else m
        return m if acc is None else jnp.maximum(acc, m)

    def a_block(rep, s, hooks):
        r0 = s * L
        use_mem = s > 0
        do_upd = s < NSEG - 1

        def hook(name):
            for f in hooks.pop(name, []):
                f()
        zparts = []
        qmx = kmx = None
        for ci, c0 in enumerate(range(0, D, NB)):
            c = slice(c0, c0 + NB)
            lhs = xa_s[r0:r0 + L, :]
            q = _dot(lhs, wq[:, c])
            qs = q * QSCALE
            q_s[:, c] = qs.astype(bf16)
            qmx = vmaxacc(qmx, qs)
            if use_mem:
                pq_s[:, c] = _phi(q).astype(bf16)
            hook(('q', ci))
            k = _dot(lhs, wk[:, c])
            k_s[:, c] = k.astype(bf16)
            kmx = vmaxacc(kmx, k)
            if do_upd:
                pk = _phi(k)
                pk_s[:, c] = pk.astype(bf16)
                zparts.append(jnp.sum(pk.reshape(L // 8, 8, NB), axis=0))
            hook(('k', ci))
            v = _dot(lhs, wv[:, c]).astype(bf16)
            vT_s[c, :] = v.T
            hook(('v', ci))
        bound = jnp.max(qmx) * jnp.max(kmx) * (DH * 1.02)
        safe = bound <= LIM
        if do_upd:
            znew = jnp.sum(jnp.concatenate(zparts, axis=1), axis=0, keepdims=True)
        for g in range(NG):
            c = slice(128 * g, 128 * (g + 1))
            if use_mem:
                m_old = mT_s[g]
                z_old = z_s[0:1, c]
                mT = jnp.where(bd, m_old, 0.0).astype(bf16)
                zr = jnp.where(zmask, jnp.broadcast_to(z_old, (32, 128)), 0.0).astype(bf16)
                lhs = jnp.concatenate([mT, zr], axis=0)
                nd_s[g] = _dot_nt(lhs, pq_s[:, c])
            if do_upd:
                upd = _dot(vT_s[c, :], pk_s[:, c])
                if use_mem:
                    mT_s[g] = m_old + upd
                    z_s[0:1, c] = z_old + znew[:, c]
                else:
                    mT_s[g] = upd
                    z_s[0:1, c] = znew[:, c]
        items = [(g, i, j) for g in range(NG) for i in IORD for j in range(i + 1)]
        st = {}
        for t in range(len(items) + DEPTH):
            if t < len(items):
                qk(st, *items[t])
            if t - DEPTH >= 0:
                pv(st, *items[t - DEPTH], use_mem)
            hook(('att', t))
        hook('att_end')

        @pl.when(jnp.logical_not(safe))
        def _():
            attn_safe_path(use_mem)
        HF = L // 2
        for r in (0, HF):
            for c0 in range(0, D, NB):
                c = slice(c0, c0 + NB)
                xres[r0 + r:r0 + r + HF, c] = xres[r0 + r:r0 + r + HF, c] + _dot(o_s[r:r + HF, :], wo[:, c])
                if r == HF and c0 == 0:
                    ln2(r0, 0, HF // 2)
                if r == HF and c0 == 2 * NB:
                    ln2(r0, HF // 2, HF // 2)
        for r in (0, HF):
            for c0 in range(0, D, NB):
                c = slice(c0, c0 + NB)
                hbuf[8 + r0 + r:8 + r0 + r + HF, c] = _gelu(_dot(xb_s[r:r + HF, :], w1[:, c]))
                if r == 0 and c0 == 0:
                    ln2(r0, HF, HF // 2)
                if r == 0 and c0 == 2 * NB:
                    ln2(r0, HF + HF // 2, HF // 2)
            hook(('w1', r))
        assert not hooks, hooks

    def b_block(final, b, hooks):
        r0 = b * L
        HF = L // 2

        def hook(name):
            for f in hooks.pop(name, []):
                f()
        for r in (0, HF):
            for c0 in range(0, D, NB):
                c = slice(c0, c0 + NB)
                x1_s[r:r + HF, c] = xn_s[r0 + r:r0 + r + HF, c] + _dot(hs_s[r0 + r:r0 + r + HF, :], w2[:, c])
                hook(('w2', r, c0))
                if r == HF and c0 == NB:
                    x1n_s[0:HF, :] = _ln(x1_s[0:HF, :]).astype(bf16)
        for c0 in range(0, F, NB):
            c = slice(c0, c0 + NB)
            if c0 == 0:
                u_s[0:HF, c] = _gelu(_dot(x1n_s[0:HF, :], w3[:, c])).astype(bf16)
                x1n_s[HF:L, :] = _ln(x1_s[HF:L, :]).astype(bf16)
                u_s[HF:L, c] = _gelu(_dot(x1n_s[HF:L, :], w3[:, c])).astype(bf16)
            else:
                u_s[:, c] = _gelu(_dot(x1n_s[...], w3[:, c])).astype(bf16)
        for c0 in range(0, D, NB4):
            c = slice(c0, c0 + NB4)
            y = xres[r0:r0 + L, c] + (x1_s[:, c] + _dot(u_s[...], w4[:, c]))
            if not final:
                xres[r0:r0 + L, c] = y
            else:
                xio[r0:r0 + L, c] = y.astype(bf16)
            hook(('w4', c0))
        assert not hooks, hooks

    def ln_a(b):
        for r in range(0, L, 256):
            rr = slice(b * L + r, b * L + r + 256)
            xa_s[rr, :] = _ln(xres[rr, :]).astype(bf16)

    def wait_w(*idx):
        for i in idx:
            w_cp[i].wait()

    x_cp[0].wait()
    w_cp[1].start()
    conv_x(0, False)
    wait_w(0)
    w_cp[2].start()
    for rep in range(NREP):
        for s in range(NSEG):
            hk = {}
            if rep == 0 and s == 0:
                hk[('q', 0)] = [lambda: wait_w(1)]
                hk[('k', 0)] = [lambda: wait_w(2), lambda: x_cp[1].start(), lambda: x_cp[2].start(), lambda: x_cp[3].start()]
                hk[('v', 0)] = [lambda: [w_cp[i].start() for i in (3, 4)]]
                hk[('v', 1)] = [lambda: conv_x(1)]
                hk[('v', 2)] = [lambda: conv_x(2)]
                hk[('v', 3)] = [lambda: conv_x(3), lambda: [w_cp[i].start() for i in (5, 6, 7)]]
                hk['att_end'] = [lambda: wait_w(3, 4)]
            if rep > 0 and s == 0:
                hk[('q', 0)] = [lambda: ln_a(3)]
            if s == NSEG - 1:
                hk[('q', 1)] = [lambda: hs_prep(0)]
                hk[('q', 2)] = [lambda: hs_prep(1)]
            args = (rep, s, hk)
            a_block(*args)
        for b in range(NSEG):
            hk = {}
            if rep == 0 and b == 0:
                wait_w(5, 6, 7)
            if b == 0:
                hk[('w2', 0, 0)] = [lambda: hs_prep(2)]
                hk[('w2', 0, NB)] = [lambda: hs_prep(3)]
            else:
                if rep < NREP - 1:
                    hk[('w2', 0, 0)] = [(lambda bb: lambda: ln_a(bb))(b - 1)]
                else:
                    hk[('w2', 0, 0)] = [(lambda bb: lambda: out_cp(bb).start())(b - 1)]
            b_block(rep == NREP - 1, b, hk)
    if NREP == 2 or True:
        out_cp(NSEG - 1).start()
        for b in range(NSEG):
            out_cp(b).wait()


@jax.jit
def pallas_interleave_layers__memory_aug_infini_attn__mixer_s_mlp__prompt_kernel(
        A_x, A_wq, A_wk, A_wv, A_wo, A_beta, B_x, B_w1, B_w2, B_w3, B_w4):
    bf16, f32 = jnp.bfloat16, jnp.float32
    V = pltpu.VMEM
    hbm = pl.BlockSpec(memory_space=pl.ANY)
    scratch = [
        V((D, D), bf16), V((D, D), bf16), V((D, D), bf16), V((D, D), bf16),
        V((D, D), bf16), V((D, D), bf16), V((D, F), bf16), V((F, D), bf16),
        V((S, D), bf16),
        V((S, D), f32),
        V((S, D), f32),
        V((S + 16, D), f32),
        V((S, D), bf16),
        V((L, D), bf16), V((L, D), bf16), V((L, D), bf16), V((L, D), bf16),
        V((D, L), bf16),
        V((L, D), bf16),
        V((L, D), bf16),
        V((NG, 128, 128), f32),
        V((8, D), f32),
        V((NG, 160, L), f32),
        V((H, 8, 128), f32),
        V((S, D), bf16),
        V((L, D), f32),
        V((L, D), bf16),
        V((L, F), bf16),
        pltpu.SemaphoreType.DMA((8,)), pltpu.SemaphoreType.DMA((NSEG,)),
        pltpu.SemaphoreType.DMA((NSEG,)),
    ]
    out = pl.pallas_call(
        _kernel,
        out_shape=jax.ShapeDtypeStruct((S, D), bf16),
        in_specs=[hbm, hbm, hbm, hbm, hbm, pl.BlockSpec(memory_space=pltpu.VMEM), hbm, hbm, hbm, hbm],
        out_specs=hbm,
        scratch_shapes=scratch,
        compiler_params=pltpu.CompilerParams(vmem_limit_bytes=120 * 2 ** 20),
        name="fused",
    )(A_x.reshape(S, D), A_wq, A_wk, A_wv, A_wo, A_beta.reshape(1, H), B_w1, B_w2, B_w3, B_w4)
    return out.reshape(1, S, D)
```
